```python
import jax
import jax.numpy as jnp

def _softmax(x, axis=-1):
    return jax.nn.softmax(x, axis=axis)
def _gelu(x):
    return jax.nn.gelu(x, approximate=True)
def _silu(x):
    return jax.nn.silu(x)
def _sigmoid(x):
    return jax.nn.sigmoid(x)
def _layernorm(x, axis=-1, eps=1e-5):
    m = jnp.mean(x, axis=axis, keepdims=True)
    v = jnp.var(x, axis=axis, keepdims=True)
    return (x - m) / jnp.sqrt(v + eps)
def _scatter_add(tgt, idx, src, axis=0):
    return tgt.at[idx].add(src)
def _segment_sum(src, seg, n):
    return jax.ops.segment_sum(src, seg, n)
class _Rng:
    def __init__(self, key):
        self._k = key
    def _next(self):
        self._k, sub = jax.random.split(self._k)
        return sub
    def normal(self, shape):
        return jax.random.normal(self._next(), shape, dtype=jnp.bfloat16)
    def randint(self, lo, hi, shape):
        return jax.random.randint(self._next(), shape, lo, hi, dtype=jnp.int32)
    def uniform(self, shape, lo=0.0, hi=1.0):
        return jax.random.uniform(self._next(), shape, jnp.bfloat16, lo, hi)
    def permutation(self, n):
        return jax.random.permutation(self._next(), n)


kernel_name = 'standalone__fused_io_aware_attn__prompt'

def setup_inputs():
    _rng = _Rng(jax.random.key(int.from_bytes(__import__("os").urandom(4), "little")))
    _w = (lambda a: (lambda t: t.astype(jnp.bfloat16) if jnp.issubdtype(t.dtype, jnp.floating) else t)(jnp.asarray(a)))
    B, H, S = 2, 32, 2048
    Dh = max(1, 1024 // 32)
    return {
        "q": _w((lambda *s: _rng.normal(s) * 0.05)(B, H, S, Dh)),
        "k": _w((lambda *s: _rng.normal(s) * 0.05)(B, H, S, Dh)),
        "v": _w((lambda *s: _rng.normal(s) * 0.05)(B, H, S, Dh)),
    }

def reference(q, k, v):
    scale = q.shape[-1] ** -0.5
    s = jnp.einsum('bhqd,bhkd->bhqk', q, k) * scale
    p = _softmax(s, axis=-1)
    return jnp.einsum('bhqk,bhkd->bhqd', p, v)
```

```python
import jax
import jax.numpy as jnp
from jax import lax
import jax.experimental.pallas as pl
import jax.experimental.pallas.tpu as pltpu

LOG2E = 1.4426950408889634
G = 4
BQ = 1024


def _attn_kernel(qt_ref, kt_ref, vt_ref, o_ref, k_scr, *, D, S):
    c = (D ** -0.5) * LOG2E
    for t in range(S // 128):
        k_scr[t * 128:(t + 1) * 128, :] = (
            kt_ref[:, t * 128:(t + 1) * 128].astype(jnp.float32).T.astype(jnp.bfloat16))

    bad = jnp.zeros((8, 128), jnp.float32)
    for h in range(G):
        for qi in range(S // BQ):
            qh = qt_ref[h * D:(h + 1) * D, qi * BQ:(qi + 1) * BQ]
            parts = []
            if h > 0:
                parts.append(jnp.zeros((h * D, BQ), jnp.bfloat16))
            parts.append(qh)
            if h < G - 1:
                parts.append(jnp.zeros(((G - 1 - h) * D, BQ), jnp.bfloat16))
            qpad = jnp.concatenate(parts, axis=0)
            s = jnp.dot(k_scr[...], qpad, preferred_element_type=jnp.float32)
            p = jnp.exp2(s * c)
            l = p.reshape(S // 8, 8, BQ).sum(axis=0)
            acc = jnp.dot(vt_ref[h * D:(h + 1) * D, :], p.astype(jnp.bfloat16),
                          preferred_element_type=jnp.float32)
            lsum = l.sum(axis=0, keepdims=True)
            o_ref[h * D:(h + 1) * D, qi * BQ:(qi + 1) * BQ] = (acc / lsum).astype(o_ref.dtype)
            okl = (lsum > 2.0 ** -30) & (lsum < 2.0 ** 100)
            oka = jnp.abs(acc) < 3.0e38
            b = jnp.where(okl & oka, 0.0, 1.0)
            b = b.reshape(D // 8, 8, BQ).max(axis=0)
            for t in range(BQ // 128):
                bad = jnp.maximum(bad, b[:, t * 128:(t + 1) * 128])

    @pl.when(jnp.max(bad) > 0.0)
    def _():
        fq, fk = 512, 512
        rowid = lax.broadcasted_iota(jnp.int32, (G * D, fq), 0)

        def one(i, _):
            h = i // (S // fq)
            qi = i % (S // fq)
            hs = pl.multiple_of(h * D, D)
            qs = pl.multiple_of(qi * fq, fq)
            q4 = qt_ref[:, pl.ds(qs, fq)]
            qpad = jnp.where((rowid >= hs) & (rowid < hs + D), q4, jnp.zeros_like(q4))

            def body(kb, carry):
                m, l, acc = carry
                ks = pl.multiple_of(kb * fk, fk)
                s = jnp.dot(k_scr[pl.ds(ks, fk), :], qpad, preferred_element_type=jnp.float32)
                m_new = jnp.maximum(m, s.max(axis=0, keepdims=True))
                alpha = jnp.exp2((m - m_new) * c)
                p = jnp.exp2((s - m_new) * c)
                l = l * alpha + p.sum(axis=0, keepdims=True)
                pv = jnp.dot(vt_ref[pl.ds(hs, D), pl.ds(ks, fk)], p.astype(jnp.bfloat16),
                             preferred_element_type=jnp.float32)
                return m_new, l, acc * alpha + pv

            init = (jnp.full((1, fq), -jnp.inf, jnp.float32),
                    jnp.zeros((1, fq), jnp.float32),
                    jnp.zeros((D, fq), jnp.float32))
            m, l, acc = lax.fori_loop(0, S // fk, body, init)
            o_ref[pl.ds(hs, D), pl.ds(qs, fq)] = (acc / l).astype(o_ref.dtype)
            return 0

        lax.fori_loop(0, G * (S // fq), one, 0)


@jax.jit
def pallas_standalone__fused_io_aware_attn__prompt_kernel(q, k, v):
    B, H, S, D = q.shape
    assert G * D == 128 and (B * H) % G == 0 and S % BQ == 0
    qt = q.transpose(0, 1, 3, 2).reshape(B * H * D, S)
    kt = k.transpose(0, 1, 3, 2).reshape(B * H * D, S)
    vt = v.transpose(0, 1, 3, 2).reshape(B * H * D, S)
    spec = pl.BlockSpec((G * D, S), lambda h: (h, 0))
    o = pl.pallas_call(
        lambda *refs: _attn_kernel(*refs, D=D, S=S),
        grid=(B * H // G,),
        in_specs=[spec, spec, spec],
        out_specs=spec,
        out_shape=jax.ShapeDtypeStruct((B * H * D, S), q.dtype),
        scratch_shapes=[pltpu.VMEM((S, G * D), jnp.bfloat16)],
        compiler_params=pltpu.CompilerParams(
            dimension_semantics=("parallel",), vmem_limit_bytes=64 * 1024 * 1024),
    )(qt, kt, vt)
    return o.reshape(B, H, D, S).transpose(0, 1, 3, 2)
```

```python
import jax
import jax.numpy as jnp
from jax import lax
import jax.experimental.pallas as pl
import jax.experimental.pallas.tpu as pltpu

LOG2E = 1.4426950408889634
G = 4
BQ = 1024


def _attn_kernel(qt_ref, kt_ref, vt_ref, o_ref, k_scr, *, D, S):
    c = (D ** -0.5) * LOG2E
    for t in range(S // 128):
        k_scr[t * 128:(t + 1) * 128, :] = (
            kt_ref[:, t * 128:(t + 1) * 128].astype(jnp.float32).T.astype(jnp.bfloat16))

    bad = jnp.zeros((8, 128), jnp.float32)
    for h in range(G):
        for qi in range(S // BQ):
            qh = qt_ref[h * D:(h + 1) * D, qi * BQ:(qi + 1) * BQ]
            parts = []
            if h > 0:
                parts.append(jnp.zeros((h * D, BQ), jnp.bfloat16))
            parts.append(qh)
            if h < G - 1:
                parts.append(jnp.zeros(((G - 1 - h) * D, BQ), jnp.bfloat16))
            qpad = jnp.concatenate(parts, axis=0)
            s = jnp.dot(k_scr[...], qpad, preferred_element_type=jnp.float32)
            p = jnp.exp2(s * c)
            l = p.reshape(S // 8, 8, BQ).sum(axis=0)
            acc = jnp.dot(vt_ref[h * D:(h + 1) * D, :], p.astype(jnp.bfloat16),
                          preferred_element_type=jnp.float32)
            lsum = l.sum(axis=0, keepdims=True)
            o_ref[h * D:(h + 1) * D, qi * BQ:(qi + 1) * BQ] = (acc / lsum).astype(o_ref.dtype)
            okl = (lsum > 2.0 ** -30) & (lsum < 2.0 ** 60)
            b = jnp.broadcast_to(jnp.where(okl, 0.0, 1.0), (8, BQ))
            if not (h == G - 1 and qi == S // BQ - 1):
                b = jnp.maximum(b, jnp.where(jnp.abs(acc) < 3.0e38, 0.0, 1.0)
                                .reshape(D // 8, 8, BQ).max(axis=0))
            for t in range(BQ // 128):
                bad = jnp.maximum(bad, b[:, t * 128:(t + 1) * 128])

    vf = jnp.abs(vt_ref[(G - 1) * D:G * D, :].astype(jnp.float32))
    vb = jnp.where(vf < 2.0 ** 60, 0.0, 1.0).reshape(D // 8, 8, S).max(axis=0)
    for t in range(S // 128):
        bad = jnp.maximum(bad, vb[:, t * 128:(t + 1) * 128])

    @pl.when(jnp.max(bad) > 0.0)
    def _():
        fq, fk = 512, 512
        rowid = lax.broadcasted_iota(jnp.int32, (G * D, fq), 0)

        def one(i, _):
            h = i // (S // fq)
            qi = i % (S // fq)
            hs = pl.multiple_of(h * D, D)
            qs = pl.multiple_of(qi * fq, fq)
            q4 = qt_ref[:, pl.ds(qs, fq)]
            qpad = jnp.where((rowid >= hs) & (rowid < hs + D), q4, jnp.zeros_like(q4))

            def body(kb, carry):
                m, l, acc = carry
                ks = pl.multiple_of(kb * fk, fk)
                s = jnp.dot(k_scr[pl.ds(ks, fk), :], qpad, preferred_element_type=jnp.float32)
                m_new = jnp.maximum(m, s.max(axis=0, keepdims=True))
                alpha = jnp.exp2((m - m_new) * c)
                p = jnp.exp2((s - m_new) * c)
                l = l * alpha + p.sum(axis=0, keepdims=True)
                pv = jnp.dot(vt_ref[pl.ds(hs, D), pl.ds(ks, fk)], p.astype(jnp.bfloat16),
                             preferred_element_type=jnp.float32)
                return m_new, l, acc * alpha + pv

            init = (jnp.full((1, fq), -jnp.inf, jnp.float32),
                    jnp.zeros((1, fq), jnp.float32),
                    jnp.zeros((D, fq), jnp.float32))
            m, l, acc = lax.fori_loop(0, S // fk, body, init)
            o_ref[pl.ds(hs, D), pl.ds(qs, fq)] = (acc / l).astype(o_ref.dtype)
            return 0

        lax.fori_loop(0, G * (S // fq), one, 0)


@jax.jit
def pallas_standalone__fused_io_aware_attn__prompt_kernel(q, k, v):
    B, H, S, D = q.shape
    assert G * D == 128 and (B * H) % G == 0 and S % BQ == 0
    qt = q.transpose(0, 1, 3, 2).reshape(B * H * D, S)
    kt = k.transpose(0, 1, 3, 2).reshape(B * H * D, S)
    vt = v.transpose(0, 1, 3, 2).reshape(B * H * D, S)
    spec = pl.BlockSpec((G * D, S), lambda h: (h, 0))
    o = pl.pallas_call(
        lambda *refs: _attn_kernel(*refs, D=D, S=S),
        grid=(B * H // G,),
        in_specs=[spec, spec, spec],
        out_specs=spec,
        out_shape=jax.ShapeDtypeStruct((B * H * D, S), q.dtype),
        scratch_shapes=[pltpu.VMEM((S, G * D), jnp.bfloat16)],
        compiler_params=pltpu.CompilerParams(
            dimension_semantics=("parallel",), vmem_limit_bytes=64 * 1024 * 1024),
    )(qt, kt, vt)
    return o.reshape(B, H, D, S).transpose(0, 1, 3, 2)
```
